```python
import jax
import jax.numpy as jnp

def _softmax(x, axis=-1):
    return jax.nn.softmax(x, axis=axis)
def _gelu(x):
    return jax.nn.gelu(x, approximate=True)
def _silu(x):
    return jax.nn.silu(x)
def _sigmoid(x):
    return jax.nn.sigmoid(x)
def _layernorm(x, axis=-1, eps=1e-5):
    m = jnp.mean(x, axis=axis, keepdims=True)
    v = jnp.var(x, axis=axis, keepdims=True)
    return (x - m) / jnp.sqrt(v + eps)
def _scatter_add(tgt, idx, src, axis=0):
    return tgt.at[idx].add(src)
def _segment_sum(src, seg, n):
    return jax.ops.segment_sum(src, seg, n)
class _Rng:
    def __init__(self, key):
        self._k = key
    def _next(self):
        self._k, sub = jax.random.split(self._k)
        return sub
    def normal(self, shape):
        return jax.random.normal(self._next(), shape, dtype=jnp.bfloat16)
    def randint(self, lo, hi, shape):
        return jax.random.randint(self._next(), shape, lo, hi, dtype=jnp.int32)
    def uniform(self, shape, lo=0.0, hi=1.0):
        return jax.random.uniform(self._next(), shape, jnp.bfloat16, lo, hi)
    def permutation(self, n):
        return jax.random.permutation(self._next(), n)


kernel_name = 'sequential_preLN__sliding_block_cached__mixer_s_mlp__decode'

def setup_inputs():
    _rng = _Rng(jax.random.key(int.from_bytes(__import__("os").urandom(4), "little")))
    _w = (lambda a: (lambda t: t.astype(jnp.bfloat16) if jnp.issubdtype(t.dtype, jnp.floating) else t)(jnp.asarray(a)))
    def _A_setup():
        B, Sq, D = 1, 1, 640
        Hq, Hkv, Sk, Dh = 32, 32, 32768, 192
        assert Hq % Hkv == 0, (Hq, Hkv)
        return {
            "x": _w((lambda *s: _rng.normal(s) * 0.05)(B, Sq, D)),
            "k_cache": _w((lambda *s: _rng.normal(s) * 0.05)(B, Hkv, Sk, Dh)),
            "v_cache": _w((lambda *s: _rng.normal(s) * 0.05)(B, Hkv, Sk, Dh)),
            "wq": _w((lambda *s: _rng.normal(s) * 0.05)(D, Hq * Dh) * (D ** -0.5)),
            "wo": _w((lambda *s: _rng.normal(s) * 0.05)(Hq * Dh, D) * ((Hq * Dh) ** -0.5)),
        }
    _A_in = _A_setup()

    def _B_setup():
        B, S, D, F = 1, 1, 640, 1536
        return {
            "x":  _w((lambda *s: _rng.normal(s) * 0.05)(B, S, D)),
            "w1": _w((lambda *s: _rng.normal(s) * 0.05)(D, D) * (D ** -0.5)),
            "w2": _w((lambda *s: _rng.normal(s) * 0.05)(D, D) * (D ** -0.5)),
            "w3": _w((lambda *s: _rng.normal(s) * 0.05)(D, F) * (D ** -0.5)),
            "w4": _w((lambda *s: _rng.normal(s) * 0.05)(F, D) * (F ** -0.5)),
        }
    _B_in = _B_setup()

    return {
        "A_x": _A_in["x"],
        "A_k_cache": _A_in["k_cache"],
        "A_v_cache": _A_in["v_cache"],
        "A_wq": _A_in["wq"],
        "A_wo": _A_in["wo"],
        "B_x": _B_in["x"],
        "B_w1": _B_in["w1"],
        "B_w2": _B_in["w2"],
        "B_w3": _B_in["w3"],
        "B_w4": _B_in["w4"],
    }

def reference(A_x, A_k_cache, A_v_cache, A_wq, A_wo, B_x, B_w1, B_w2, B_w3, B_w4):
    def _A_ref(x, k_cache, v_cache, wq, wo):
        B, Sq, D = x.shape
        Hq, Dh = 32, 192
        Hkv, Sk = k_cache.shape[1], k_cache.shape[2]
        W = min(4096, max(256, Sk // 4))
        rep = Hq // Hkv
        q = (lambda x, *d: x.transpose(*d))((x @ wq).reshape(B, Sq, Hq, Dh), 0, 2, 1, 3)
        k = jnp.repeat(k_cache[:, :, Sk - W:, :], rep, axis=1)
        v = jnp.repeat(v_cache[:, :, Sk - W:, :], rep, axis=1)
        scores = jnp.einsum("bhqd,bhkd->bhqk", q, k) * (Dh ** -0.5)
        p = _softmax(scores, axis=-1)
        o = jnp.einsum("bhqk,bhkd->bhqd", p, v)
        return (lambda x, *d: x.transpose(*d))(o, 0, 2, 1, 3).reshape(B, Sq, Hq * Dh) @ wo

    def _B_ref(x, w1, w2, w3, w4):
        B, S, D = x.shape
        h = _gelu(_layernorm(x, axis=-1) @ w1)
        c = D // 4
        g0 = jnp.pad(h[:, :, 0*c:1*c], ((0, 0), (1, 0), (0, 0)))[:, :S, :]
        g1 = jnp.pad(h[:, :, 1*c:2*c], ((0, 0), (0, 1), (0, 0)))[:, 1:, :]
        g2 = jnp.pad(h[:, :, 2*c:3*c], ((0, 0), (2, 0), (0, 0)))[:, :S, :]
        g3 = jnp.pad(h[:, :, 3*c:   ], ((0, 0), (0, 2), (0, 0)))[:, 2:, :]
        hs = jnp.concatenate([g0, g1, g2, g3], axis=-1) @ w2
        x1 = x + hs
        h2 = _gelu(_layernorm(x1, axis=-1) @ w3) @ w4
        return x1 + h2

    x = A_x
    h = x + _A_ref(_layernorm(x, axis=-1), A_k_cache, A_v_cache, A_wq, A_wo)
    h2 = h + _B_ref(_layernorm(h, axis=-1), B_w1, B_w2, B_w3, B_w4)
    return h2
```

```python
import jax
import jax.numpy as jnp
from jax import lax
import jax.experimental.pallas as pl
import jax.experimental.pallas.tpu as pltpu

_EPS = 1e-5
_NB = 4
_MR = 8


def _layernorm(x):
    m = jnp.mean(x, axis=-1, keepdims=True)
    xc = x - m
    v = jnp.mean(xc * xc, axis=-1, keepdims=True)
    return xc * lax.rsqrt(v + _EPS)


def _make_kernel(D, H, DH, SK, W, F):
    NP = H // 2
    PW = 2 * DH
    NB, MR = _NB, _MR

    def kern(x_ref, k_hbm, v_hbm, wq_hbm, wo_hbm, w3_hbm, w4_hbm, o_ref,
             kb, vb, wqb, wob, w3b, w4b, qbd, sk, sv, sw):
        def kcp(j, slot):
            return pltpu.make_async_copy(
                k_hbm.at[pl.ds(j * PW, PW), pl.ds(SK - W, W)], kb.at[slot], sk.at[slot])

        def vcp(j, slot):
            return pltpu.make_async_copy(
                v_hbm.at[pl.ds(j * PW, PW), pl.ds(SK - W, W)], vb.at[slot], sv.at[slot])

        wq_cp = pltpu.make_async_copy(wq_hbm, wqb, sw.at[0])
        wo_cp = pltpu.make_async_copy(wo_hbm, wob, sw.at[1])
        w3_cp = pltpu.make_async_copy(w3_hbm, w3b, sw.at[2])
        w4_cp = pltpu.make_async_copy(w4_hbm, w4b, sw.at[3])
        wq_cp.start()
        wo_cp.start()
        for j in range(NB):
            kcp(j, j).start()
            vcp(j, j).start()

        x = x_ref[...].astype(jnp.float32)
        xn = _layernorm(x).astype(jnp.bfloat16)
        xn8 = jnp.broadcast_to(xn, (MR, D))
        wq_cp.wait()
        row = lax.broadcasted_iota(jnp.int32, (MR, PW), 0)
        col = lax.broadcasted_iota(jnp.int32, (MR, PW), 1)
        mask = (col >= row * DH) & (col < (row + 1) * DH)
        for j in range(NP):
            q = jnp.dot(xn8, wqb[:, j * PW:(j + 1) * PW], preferred_element_type=jnp.float32)
            qbd[j] = jnp.where(mask, q, 0.0).astype(jnp.bfloat16)
        wo_cp.wait()
        scale = DH ** -0.5

        def body(j, acc):
            slot = j % NB
            kcp(j, slot).wait()
            s = jnp.dot(qbd[j], kb[slot], preferred_element_type=jnp.float32) * scale

            @pl.when(j + NB < NP)
            def _():
                kcp(j + NB, slot).start()

            m = jnp.max(s, axis=-1, keepdims=True)
            e = jnp.exp(s - m)
            l = jnp.sum(e, axis=-1, keepdims=True)
            vcp(j, slot).wait()
            o = lax.dot_general(e.astype(jnp.bfloat16), vb[slot], (((1,), (1,)), ((), ())),
                                preferred_element_type=jnp.float32)

            @pl.when(j + NB < NP)
            def _():
                vcp(j + NB, slot).start()

            @pl.when(j + NB == NP - 1)
            def _():
                w3_cp.start()
                w4_cp.start()

            o = jnp.where(mask, o / l, 0.0).astype(jnp.bfloat16)
            return acc + jnp.dot(o, wob[j], preferred_element_type=jnp.float32)

        acc = lax.fori_loop(0, NP, body, jnp.zeros((MR, D), jnp.float32))
        attn = jnp.sum(acc, axis=0, keepdims=True)
        h = x + attn
        xb = _layernorm(h)
        y = _layernorm(xb).astype(jnp.bfloat16)
        w3_cp.wait()
        z = jnp.dot(jnp.broadcast_to(y, (MR, D)), w3b[...], preferred_element_type=jnp.float32)
        g = jax.nn.gelu(z, approximate=True).astype(jnp.bfloat16)
        w4_cp.wait()
        h2 = jnp.dot(g, w4b[...], preferred_element_type=jnp.float32)[0:1]
        o_ref[...] = (h + xb + h2).astype(o_ref.dtype)

    return kern


@jax.jit
def pallas_sequential_preLN__sliding_block_cached__mixer_s_mlp__decode_kernel(
    A_x: jax.Array,
    A_k_cache: jax.Array,
    A_v_cache: jax.Array,
    A_wq: jax.Array,
    A_wo: jax.Array,
    B_x: jax.Array,
    B_w1: jax.Array,
    B_w2: jax.Array,
    B_w3: jax.Array,
    B_w4: jax.Array,
):
    B, Sq, D = A_x.shape
    _, H, SK, DH = A_k_cache.shape
    F = B_w3.shape[1]
    W = min(4096, max(256, SK // 4))
    assert B == 1 and Sq == 1 and H % 2 == 0
    NP, PW = H // 2, 2 * DH

    kt = jnp.swapaxes(A_k_cache, 2, 3).reshape(H * DH, SK)
    vt = jnp.swapaxes(A_v_cache, 2, 3).reshape(H * DH, SK)
    any_spec = pl.BlockSpec(memory_space=pl.ANY)
    bf = jnp.bfloat16
    out = pl.pallas_call(
        _make_kernel(D, H, DH, SK, W, F),
        out_shape=jax.ShapeDtypeStruct((1, D), A_x.dtype),
        in_specs=[pl.BlockSpec(memory_space=pltpu.VMEM)] + [any_spec] * 6,
        out_specs=pl.BlockSpec(memory_space=pltpu.VMEM),
        scratch_shapes=[
            pltpu.VMEM((_NB, PW, W), bf),
            pltpu.VMEM((_NB, PW, W), bf),
            pltpu.VMEM((D, H * DH), bf),
            pltpu.VMEM((NP, PW, D), bf),
            pltpu.VMEM((D, F), bf),
            pltpu.VMEM((F, D), bf),
            pltpu.VMEM((NP, _MR, PW), bf),
            pltpu.SemaphoreType.DMA((_NB,)),
            pltpu.SemaphoreType.DMA((_NB,)),
            pltpu.SemaphoreType.DMA((4,)),
        ],
        compiler_params=pltpu.CompilerParams(vmem_limit_bytes=100 * 1024 * 1024),
    )(A_x.reshape(1, D), kt, vt, A_wq, A_wo.reshape(NP, PW, D), B_w3, B_w4)
    return out.reshape(1, 1, D)
```

```python
import jax
import jax.numpy as jnp
from jax import lax
import jax.experimental.pallas as pl
import jax.experimental.pallas.tpu as pltpu

D=640; H=32; DH=192; SK=32768; W=4096; F=1536
NP = H//2
PW = 2*DH
EPS=1e-5

def _ln(x):
    m = jnp.mean(x, axis=-1, keepdims=True)
    xc = x - m
    v = jnp.mean(xc*xc, axis=-1, keepdims=True)
    return xc * lax.rsqrt(v + EPS)

def _make(DEP=7, MR=8, WOR=16, WOS=2, W3C=768, W4R=16, PW4=6, nobounds=True, prios=(0,1), w4at=0, nocomp=False):
    CL = 24 + WOS
    NQ = 30
    PAN = 1024
    def kern(x_hbm, k_hbm, v_hbm, wq_hbm, wo_hbm, w3_hbm, w4_hbm, o_ref,
             xb_, kb, vb, wqb, wob, w3b, w4b, qbd, sx, sq, sp, sw3, sw4):
        def pr(i): return prios[i % len(prios)]
        def wq_start(g):
            c, r = g // 5, g % 5
            for i in range(16):
                r0 = 128*r + 8*i
                pltpu.make_async_copy(wq_hbm.at[pl.ds(r0, 8), pl.ds(PAN*c, PAN)], wqb.at[pl.ds(r0, 8), pl.ds(PAN*c, PAN)], sq.at[g]).start(priority=pr(i))
        def wq_wait(g):
            c, r = g // 5, g % 5
            d = wqb.at[pl.ds(128*r, 128), pl.ds(PAN*c, PAN)]
            pltpu.make_async_copy(d, d, sq.at[g]).wait()
        def sub_start(j, u):
            if u < 24:
                src, buf = (k_hbm, kb) if u < 12 else (v_hbm, vb)
                p, r = (u % 12) // 3, u % 3
                base = pl.multiple_of(j * PW, 8)
                for i in range(16):
                    r0 = 128*r + 8*i
                    pltpu.make_async_copy(src.at[pl.ds(base + r0, 8), pl.ds(SK - W + PAN*p, PAN)], buf.at[pl.ds(r0, 8), pl.ds(PAN*p, PAN)], sp.at[u]).start(priority=pr(i))
            else:
                s = u - 24
                n = PW // WOS
                base = pl.multiple_of(j * PW, 8)
                for i in range(n // WOR):
                    r0 = n*s + WOR*i
                    pltpu.make_async_copy(wo_hbm.at[pl.ds(base + r0, WOR)], wob.at[pl.ds(r0, WOR)], sp.at[u]).start(priority=pr(i))
        def sub_wait(u):
            if u < 24:
                buf = kb if u < 12 else vb
                p, r = (u % 12) // 3, u % 3
                d = buf.at[pl.ds(128*r, 128), pl.ds(PAN*p, PAN)]
            else:
                s = u - 24
                n = PW // WOS
                d = wob.at[pl.ds(n*s, n)]
            pltpu.make_async_copy(d, d, sp.at[u]).wait()
        def w3_start():
            nc = F // W3C
            def st(i, c):
                r0 = pl.multiple_of((i // nc) * 8, 8); c0 = pl.multiple_of((i % nc) * W3C, 128)
                for k in range(2):
                    r1 = pl.multiple_of(r0 + k * 8 * (D // 16), 8)
                    pltpu.make_async_copy(w3_hbm.at[pl.ds(r1, 8), pl.ds(c0, W3C)], w3b.at[pl.ds(r1, 8), pl.ds(c0, W3C)], sw3).start(priority=pr(k))
                return c
            lax.fori_loop(0, (D // 16) * nc, st, 0)
        r4 = F // PW4
        def w4_start():
            def st(i, c):
                cc = i // (r4 // W4R // 2)
                for k in range(2):
                    r1 = pl.multiple_of((2*i + k) * W4R, 8)
                    pltpu.make_async_copy(w4_hbm.at[pl.ds(r1, W4R)], w4b.at[pl.ds(r1, W4R)], sw4.at[cc]).start(priority=pr(k))
                return c
            lax.fori_loop(0, F // W4R // 2, st, 0)

        x_cp = pltpu.make_async_copy(x_hbm, xb_, sx)
        x_cp.start()
        for g in range(DEP): wq_start(g)
        x_cp.wait()
        x = xb_[...].astype(jnp.float32)
        xn = _ln(x).astype(jnp.bfloat16)
        xn8 = jnp.broadcast_to(xn, (MR, D))
        row = lax.broadcasted_iota(jnp.int32, (MR, PW), 0)
        col = lax.broadcasted_iota(jnp.int32, (MR, PW), 1)
        mask = (col >= row*DH) & (col < (row+1)*DH)
        for g in range(NQ):
            wq_wait(g)
            t = g + DEP
            if t < NQ: wq_start(t)
            else: sub_start(0, t - NQ)
            if g % 5 == 4 and not nocomp:
                c = g // 5
                q = jnp.dot(xn8, wqb[:, c*PAN:(c+1)*PAN], preferred_element_type=jnp.float32)
                for k in range(8):
                    ti = 8*c + k
                    j, kk = ti // 3, ti % 3
                    qbd[j, :, 128*kk:128*(kk+1)] = jnp.where(mask[:, 128*kk:128*(kk+1)], q[:, 128*k:128*(k+1)], 0.0).astype(jnp.bfloat16)
        scale = DH ** -0.5
        def body(j, acc):
            s = []
            e = None
            o = jnp.zeros((MR, PW), jnp.float32)
            for u in range(CL):
                sub_wait(u)
                t = u + DEP
                if t < CL:
                    sub_start(j, t)
                else:
                    @pl.when(j + 1 < NP)
                    def _():
                        sub_start(j + 1, t - CL)
                    if t == CL:
                        @pl.when(j + 1 == NP)
                        def _():
                            w3_start()
                    if t == CL + w4at or (u == CL - 1 and CL + w4at > t):
                        @pl.when(j + 1 == NP)
                        def _():
                            w4_start()
                if nocomp: continue
                if u < 12 and u % 3 == 2:
                    p = u // 3
                    s.append(jnp.dot(qbd[j], kb[:, p*PAN:(p+1)*PAN], preferred_element_type=jnp.float32) * scale)
                    if p == 3:
                        m = jnp.maximum(jnp.maximum(s[0], s[1]), jnp.maximum(s[2], s[3]))
                        m = jnp.max(m, axis=-1, keepdims=True)
                        ef = [jnp.exp(x - m) for x in s]
                        l = jnp.sum((ef[0] + ef[1]) + (ef[2] + ef[3]), axis=-1, keepdims=True)
                        e = [x.astype(jnp.bfloat16) for x in ef]
                elif 12 <= u < 24 and u % 3 == 2:
                    p = (u - 12) // 3
                    o = o + lax.dot_general(e[p], vb[:, p*PAN:(p+1)*PAN], (((1,),(1,)),((),())), preferred_element_type=jnp.float32)
                elif u == CL - 1:
                    ob = jnp.where(mask, o / l, 0.0).astype(jnp.bfloat16)
                    acc = acc + jnp.dot(ob, wob[...], preferred_element_type=jnp.float32)
            return acc
        acc = lax.fori_loop(0, NP, body, jnp.zeros((MR, D), jnp.float32))
        attn = jnp.sum(acc, axis=0, keepdims=True)
        h = x + attn
        xb = _ln(h)
        y = _ln(xb).astype(jnp.bfloat16)
        pltpu.make_async_copy(w3b, w3b, sw3).wait()
        z = jnp.dot(jnp.broadcast_to(y, (MR, D)), w3b[...], preferred_element_type=jnp.float32)
        g = jax.nn.gelu(z, approximate=True).astype(jnp.bfloat16)
        h2 = jnp.broadcast_to(h + xb, (MR, D))
        for c in range(PW4):
            d = w4b.at[pl.ds(c*r4, r4)]
            pltpu.make_async_copy(d, d, sw4.at[c]).wait()
            h2 = h2 + jnp.dot(g[:, c*r4:(c+1)*r4], w4b[c*r4:(c+1)*r4, :], preferred_element_type=jnp.float32)
        o_ref[...] = h2[0:1].astype(jnp.bfloat16)

    def fn(A_x, A_k_cache, A_v_cache, A_wq, A_wo, B_x, B_w1, B_w2, B_w3, B_w4):
        kt = jnp.swapaxes(A_k_cache, 2, 3).reshape(H*DH, SK)
        vt = jnp.swapaxes(A_v_cache, 2, 3).reshape(H*DH, SK)
        any_ = pl.BlockSpec(memory_space=pl.ANY)
        DMA = pltpu.SemaphoreType.DMA
        out = pl.pallas_call(kern,
            out_shape=jax.ShapeDtypeStruct((1,D), jnp.bfloat16),
            in_specs=[any_]*7,
            out_specs=pl.BlockSpec(memory_space=pltpu.VMEM),
            scratch_shapes=[pltpu.VMEM((1,D), jnp.bfloat16), pltpu.VMEM((PW,W), jnp.bfloat16), pltpu.VMEM((PW,W), jnp.bfloat16),
              pltpu.VMEM((D,H*DH), jnp.bfloat16), pltpu.VMEM((PW,D), jnp.bfloat16), pltpu.VMEM((D,F), jnp.bfloat16), pltpu.VMEM((F,D), jnp.bfloat16),
              pltpu.VMEM((NP,MR,PW), jnp.bfloat16),
              DMA(()), DMA((NQ,)), DMA((CL,)), DMA(()), DMA((PW4,))],
            compiler_params=pltpu.CompilerParams(vmem_limit_bytes=64*1024*1024, disable_bounds_checks=nobounds),
        )(A_x.reshape(1,D), kt, vt, A_wq, A_wo, B_w3, B_w4)
        return out.reshape(1,1,D)
    return fn


_fn = _make(DEP=6)


@jax.jit
def pallas_sequential_preLN__sliding_block_cached__mixer_s_mlp__decode_kernel(
    A_x, A_k_cache, A_v_cache, A_wq, A_wo, B_x, B_w1, B_w2, B_w3, B_w4
):
    return _fn(A_x, A_k_cache, A_v_cache, A_wq, A_wo, B_x, B_w1, B_w2, B_w3, B_w4)
```

```python
import jax
import jax.numpy as jnp
from jax import lax
import jax.experimental.pallas as pl
import jax.experimental.pallas.tpu as pltpu

D=640; H=32; DH=192; SK=32768; W=4096; F=1536
NP = H//2
PW = 2*DH
EPS=1e-5
PAN=1024; NPAN=W//PAN

def _ln(x):
    m = jnp.mean(x, axis=-1, keepdims=True)
    xc = x - m
    v = jnp.mean(xc*xc, axis=-1, keepdims=True)
    return xc * lax.rsqrt(v + EPS)

def loop(n, f, lo=0, unroll=1):
    def b(i, c):
        f(i); return c
    lax.fori_loop(lo, n, b, 0, unroll=unroll)

def _make(MR=8, QDEP=5, ODEP=7, woS=32, won=12, nocomp=False, cp=(1,1,1), PW4=6, w3S=10, qat=4, unr=1, kvunr=1, wunr=1, pr0=0):
    DEP = 4
    NQ = 24; QS = 20
    NO = 384 // won
    r4 = F // PW4
    N3P = 80; N4P = 96
    QR = QDEP + 1; ORING = ODEP + 1

    def kern(x_hbm, k_hbm, v_hbm, wq_hbm, wo_hbm, w3_hbm, w4_hbm, o_ref,
             xb_, kb, vb, wqb, wob, w3b, w4b, qbd, ssc, esc, gsc, sx, sq, so, sp, s3, s4):
        m8 = lambda v: pl.multiple_of(v, 8)
        def wq_cps(g):
            s = g % QR
            rb = m8((g // 3) * 8); cb = pl.multiple_of((g % 3) * (2*PAN), 128)
            return [pltpu.make_async_copy(wq_hbm.at[pl.ds(rb + 64*m, 8), pl.ds(cb + PAN*par, PAN)], wqb.at[pl.ds(rb + 64*m, 8), pl.ds(cb + PAN*par, PAN)], sq.at[s])
                    for m in range(10) for par in range(2)]
        def wq_start(g):
            for i, c in enumerate(wq_cps(g)): c.start(priority=i % 2)
        def wq_wait(g):
            for c in wq_cps(g): c.wait()
        def wo_cps(g):
            s = g % ORING
            rb = m8(g * 16)
            return [pltpu.make_async_copy(wo_hbm.at[pl.ds(rb + 16*woS*n, 16)], wob.at[pl.ds(rb + 16*woS*n, 16)], so.at[s]) for n in range(won)]
        def wo_start(g):
            for i, c in enumerate(wo_cps(g)): c.start(priority=i % 2)
        def wo_wait(g):
            for c in wo_cps(g): c.wait()
        def kv_cp(isv, j, p, h, i):
            src, buf = (v_hbm, vb) if isv else (k_hbm, kb)
            c0 = pl.multiple_of(SK - W + p * PAN, 128)
            r0 = m8(8*h + 16*i)
            return pltpu.make_async_copy(src.at[pl.ds(m8(j * PW + r0), 8), pl.ds(c0, PAN)], buf.at[p, i, pl.ds(m8(8*h), 8)], sp.at[int(isv), p, h])
        def kv_start(isv, j, p, h):
            def st(i):
                kv_cp(isv, j, p, h, 2*i).start(priority=pr0)
                kv_cp(isv, j, p, h, 2*i + 1).start(priority=1 - pr0)
            loop(12, st, unroll=kvunr)
        def kv_wait(isv, j, p, h):
            buf = vb if isv else kb
            d = buf.at[p, :, pl.ds(m8(8*h), 8)]
            pltpu.make_async_copy(d, d, sp.at[int(isv), p, h]).wait()
        def w3_start(i0, i1):
            per3 = N3P // w3S
            def st(ii):
                for k in range(2):
                    i = 2*ii + k
                    tr = (i // per3) + w3S * (i % per3)
                    r1 = m8(tr * 8)
                    pltpu.make_async_copy(w3_hbm.at[pl.ds(r1, 8)], w3b.at[pl.ds(r1, 8)], s3).start(priority=k)
            loop(i1, st, lo=i0)
        def w4_start(i0, i1):
            n = r4 // 16
            def st(ii):
                c = ii // (n // 2); w = ii % (n // 2)
                for k in range(2):
                    r1 = m8((w + k*(n//2)) * 16)
                    pltpu.make_async_copy(w4_hbm.at[c, pl.ds(r1, 16)], w4b.at[c, pl.ds(r1, 16)], s4.at[c]).start(priority=k)
            loop(i1, st, lo=i0)

        x_cp = pltpu.make_async_copy(x_hbm, xb_, sx)
        x_cp.start()
        loop(QDEP, wq_start)
        x_cp.wait()
        x = xb_[...].astype(jnp.float32)
        xn = _ln(x).astype(jnp.bfloat16)
        xn8 = jnp.broadcast_to(xn, (MR, D))
        def a(g):
            wq_wait(g); wq_start(g + QDEP)
        loop(NQ - QDEP, a)
        def b(g):
            wq_wait(g); wo_start(g - (NQ - QDEP))
        loop(NQ, b, lo=NQ - QDEP)
        loop(ODEP, wo_start, lo=QDEP)
        row = lax.broadcasted_iota(jnp.int32, (MR, 128), 0)
        col = lax.broadcasted_iota(jnp.int32, (MR, 128), 1)
        def qproj(c):
            q = jnp.dot(xn8, wqb[:, pl.ds(pl.multiple_of(c*PAN, 128), PAN)], preferred_element_type=jnp.float32)
            for k in range(8):
                ti = 8*c + k
                cc = col + 128 * (ti % 3)
                mk = (cc >= row*DH) & (cc < (row+1)*DH)
                qbd[ti] = jnp.where(mk, q[:, 128*k:128*(k+1)], 0.0).astype(jnp.bfloat16)
        def c_(g):
            wo_wait(g)
            @pl.when(g + ODEP < NO)
            def _(): wo_start(g + ODEP)
            @pl.when(g + DEP >= NO)
            def _():
                u = g + DEP - NO
                kv_start(False, 0, u // 2, u % 2)
            if not nocomp and cp[0]:
                @pl.when((g % qat == 0) & (g < 6*qat))
                def _(): qproj(g // qat)
        loop(NO, c_)
        rowp = lax.broadcasted_iota(jnp.int32, (MR, PW), 0)
        colp = lax.broadcasted_iota(jnp.int32, (MR, PW), 1)
        maskp = (colp >= rowp*DH) & (colp < (rowp+1)*DH)
        scale = DH ** -0.5
        NT = (N3P + N4P) // 2
        def body(j, acc):
            def kstep(p):
                for r in range(2):
                    kv_wait(False, j, p, r)
                    @pl.when(p < 2)
                    def _(): kv_start(False, j, p + 2, r)
                    @pl.when(p >= 2)
                    def _(): kv_start(True, j, p - 2, r)
                if not nocomp and cp[1]:
                    q3 = jnp.concatenate([qbd[3*j], qbd[3*j+1], qbd[3*j+2]], axis=1)
                    ssc[p] = jnp.dot(q3, kb[p].reshape(PW, PAN), preferred_element_type=jnp.float32) * scale
            loop(NPAN, kstep)
            if not nocomp and cp[1]:
                s = [ssc[p] for p in range(NPAN)]
                m = jnp.maximum(jnp.maximum(s[0], s[1]), jnp.maximum(s[2], s[3]))
                m = jnp.max(m, axis=-1, keepdims=True)
                ef = [jnp.exp(x - m) for x in s]
                l = jnp.sum((ef[0] + ef[1]) + (ef[2] + ef[3]), axis=-1, keepdims=True)
                for p in range(NPAN): esc[p] = ef[p].astype(jnp.bfloat16)
            def vstep(p, o):
                for r in range(2):
                    kv_wait(True, j, p, r)
                    @pl.when(p < 2)
                    def _(): kv_start(True, j, p + 2, r)
                    @pl.when((p >= 2) & (j + 1 < NP))
                    def _(): kv_start(False, j + 1, p - 2, r)
                    @pl.when((p >= 2) & (j + 1 == NP))
                    def _():
                        v = (p - 2) * 2 + r
                        lo = (NT * v) // DEP; hi = (NT * (v + 1)) // DEP
                        w3_start(jnp.minimum(lo, N3P//2), jnp.minimum(hi, N3P//2))
                        w4_start(jnp.maximum(lo - N3P//2, 0), jnp.maximum(hi - N3P//2, 0))
                if not nocomp and cp[1]:
                    o = o + lax.dot_general(esc[p], vb[p].reshape(PW, PAN), (((1,),(1,)),((),())), preferred_element_type=jnp.float32)
                return o
            o = lax.fori_loop(0, NPAN, vstep, jnp.zeros((MR, PW), jnp.float32))
            if not nocomp and cp[1]:
                ob = jnp.where(maskp, o / l, 0.0).astype(jnp.bfloat16)
                acc = acc + jnp.dot(ob, wob[pl.ds(pl.multiple_of(j*PW, 16), PW), :], preferred_element_type=jnp.float32)
            return acc
        acc = lax.fori_loop(0, NP, body, jnp.zeros((MR, D), jnp.float32))
        if nocomp or not cp[2]:
            pltpu.make_async_copy(w3b, w3b, s3).wait()
            for c in range(PW4):
                pltpu.make_async_copy(w4b.at[c], w4b.at[c], s4.at[c]).wait()
            o_ref[...] = acc[0:1].astype(jnp.bfloat16)
            return
        attn = jnp.sum(acc, axis=0, keepdims=True)
        h = x + attn
        xb = _ln(h)
        y = _ln(xb).astype(jnp.bfloat16)
        pltpu.make_async_copy(w3b, w3b, s3).wait()
        z = jnp.dot(jnp.broadcast_to(y, (MR, D)), w3b[...], preferred_element_type=jnp.float32)
        g = jax.nn.gelu(z, approximate=True).astype(jnp.bfloat16)
        for c in range(PW4): gsc[c] = g[:, c*r4:(c+1)*r4]
        def fin(c, h2):
            pltpu.make_async_copy(w4b.at[c], w4b.at[c], s4.at[c]).wait()
            return h2 + jnp.dot(gsc[c], w4b[c], preferred_element_type=jnp.float32)
        h2 = lax.fori_loop(0, PW4, fin, jnp.broadcast_to(h + xb, (MR, D)))
        o_ref[...] = h2[0:1].astype(jnp.bfloat16)

    def fn(A_x, A_k_cache, A_v_cache, A_wq, A_wo, B_x, B_w1, B_w2, B_w3, B_w4):
        kt = jnp.swapaxes(A_k_cache, 2, 3).reshape(H*DH, SK)
        vt = jnp.swapaxes(A_v_cache, 2, 3).reshape(H*DH, SK)
        any_ = pl.BlockSpec(memory_space=pl.ANY)
        DMA = pltpu.SemaphoreType.DMA
        out = pl.pallas_call(kern,
            out_shape=jax.ShapeDtypeStruct((1,D), jnp.bfloat16),
            in_specs=[any_]*7,
            out_specs=pl.BlockSpec(memory_space=pltpu.VMEM),
            scratch_shapes=[pltpu.VMEM((1,D), jnp.bfloat16), pltpu.VMEM((NPAN,PW//16,16,PAN), jnp.bfloat16), pltpu.VMEM((NPAN,PW//16,16,PAN), jnp.bfloat16),
              pltpu.VMEM((D,H*DH), jnp.bfloat16), pltpu.VMEM((H*DH,D), jnp.bfloat16), pltpu.VMEM((D,F), jnp.bfloat16), pltpu.VMEM((PW4,r4,D), jnp.bfloat16),
              pltpu.VMEM((48,MR,128), jnp.bfloat16), pltpu.VMEM((NPAN,MR,PAN), jnp.float32), pltpu.VMEM((NPAN,MR,PAN), jnp.bfloat16), pltpu.VMEM((PW4,MR,r4), jnp.bfloat16),
              DMA(()), DMA((QR,)), DMA((ORING,)), DMA((2,NPAN,2)), DMA(()), DMA((PW4,))],
            compiler_params=pltpu.CompilerParams(vmem_limit_bytes=64*1024*1024, disable_bounds_checks=True),
        )(A_x.reshape(1,D), kt, vt, A_wq, A_wo, B_w3, B_w4.reshape(PW4, r4, D))
        return out.reshape(1,1,D)
    return fn


_fn = _make(kvunr=2)


@jax.jit
def pallas_sequential_preLN__sliding_block_cached__mixer_s_mlp__decode_kernel(
    A_x, A_k_cache, A_v_cache, A_wq, A_wo, B_x, B_w1, B_w2, B_w3, B_w4
):
    return _fn(A_x, A_k_cache, A_v_cache, A_wq, A_wo, B_x, B_w1, B_w2, B_w3, B_w4)
```

```python
import jax
import jax.numpy as jnp
from jax import lax
import jax.experimental.pallas as pl
import jax.experimental.pallas.tpu as pltpu

_EPS = 1e-5
_MR = 8
_PAN = 1024
_W4_CHUNKS = 6
_Q_DEPTH = 5
_O_DEPTH = 7
_KV_DEPTH = 4
_Q_EVERY = 4


def _layernorm(x):
    m = jnp.mean(x, axis=-1, keepdims=True)
    xc = x - m
    v = jnp.mean(xc * xc, axis=-1, keepdims=True)
    return xc * lax.rsqrt(v + _EPS)


def _loop(lo, hi, f, unroll=1):
    def body(i, carry):
        f(i)
        return carry

    lax.fori_loop(lo, hi, body, 0, unroll=unroll)


def _dot(a, b):
    return jnp.dot(a, b, preferred_element_type=jnp.float32)


def _make_kernel(D, H, DH, SK, W, F):
    NP = H // 2
    PW = 2 * DH
    MR, PAN = _MR, _PAN
    NPAN = W // PAN
    KV_PIECES = PW // 16
    QPAN = H * DH // PAN
    Q_STRIP = D // 64
    NQ = 8 * QPAN // 2
    O_PIECES = 12
    O_STRIDE = H * DH // 16 // O_PIECES
    NO = O_STRIDE
    R4 = F // _W4_CHUNKS
    W3_STRIDE = 10
    N3, N4 = D // 16, F // 32
    QD, OD, KD = _Q_DEPTH, _O_DEPTH, _KV_DEPTH
    assert NPAN == 4 and KD == 4 and PW % 128 == 0 and PW % 16 == 0
    assert D % 128 == 0 and QPAN == 6 and D // 8 % W3_STRIDE == 0 and R4 % 32 == 0
    assert O_STRIDE * O_PIECES * 16 == H * DH and QD <= OD <= NO - _Q_EVERY * QPAN

    def m8(v):
        return pl.multiple_of(v, 8)

    def m128(v):
        return pl.multiple_of(v, 128)

    def kernel(x_hbm, k_hbm, v_hbm, wq_hbm, wo_hbm, w3_hbm, w4_hbm, o_ref,
               x_buf, k_buf, v_buf, wq_buf, wo_buf, w3_buf, w4_buf, q_buf, s_buf, p_buf, g_buf,
               x_sem, wq_sem, wo_sem, kv_sem, w3_sem, w4_sem):
        def wq_copies(g):
            r0, c0 = m8((g // 3) * 8), m128((g % 3) * (2 * PAN))
            sem = wq_sem.at[g % (QD + 1)]
            return [
                pltpu.make_async_copy(
                    wq_hbm.at[pl.ds(r0 + 64 * m, 8), pl.ds(c0 + PAN * k, PAN)],
                    wq_buf.at[pl.ds(r0 + 64 * m, 8), pl.ds(c0 + PAN * k, PAN)], sem)
                for k in range(2) for m in range(Q_STRIP)
            ]

        def wo_copies(g):
            r0 = m8(g * 16)
            sem = wo_sem.at[g % (OD + 1)]
            return [
                pltpu.make_async_copy(wo_hbm.at[pl.ds(r0 + 16 * O_STRIDE * n, 16)],
                                      wo_buf.at[pl.ds(r0 + 16 * O_STRIDE * n, 16)], sem)
                for n in range(O_PIECES)
            ]

        def start_all(copies):
            for i, c in enumerate(copies):
                c.start(priority=i % 2)

        def wait_all(copies):
            for c in copies:
                c.wait()

        def kv_start(is_v, j, p, h):
            src, buf = (v_hbm, v_buf) if is_v else (k_hbm, k_buf)
            c0 = m128(SK - W + p * PAN)
            sem = kv_sem.at[int(is_v), p, h]

            def two_pieces(i):
                for k in range(2):
                    n = 2 * i + k
                    pltpu.make_async_copy(
                        src.at[pl.ds(m8(j * PW + 16 * n + 8 * h), 8), pl.ds(c0, PAN)],
                        buf.at[p, n, pl.ds(m8(8 * h), 8)], sem).start(priority=k)

            _loop(0, KV_PIECES // 2, two_pieces)

        def kv_wait(is_v, p, h):
            dst = (v_buf if is_v else k_buf).at[p, :, pl.ds(m8(8 * h), 8)]
            pltpu.make_async_copy(dst, dst, kv_sem.at[int(is_v), p, h]).wait()

        def w3_start(lo, hi):
            per = D // 8 // W3_STRIDE

            def two_pieces(i):
                for k in range(2):
                    n = 2 * i + k
                    r0 = m8((n // per + W3_STRIDE * (n % per)) * 8)
                    pltpu.make_async_copy(w3_hbm.at[pl.ds(r0, 8)], w3_buf.at[pl.ds(r0, 8)],
                                          w3_sem).start(priority=k)

            _loop(lo, hi, two_pieces)

        def w4_start(lo, hi):
            half = R4 // 32

            def two_pieces(i):
                c = i // half
                for k in range(2):
                    r0 = m8((i % half + k * half) * 16)
                    pltpu.make_async_copy(w4_hbm.at[c, pl.ds(r0, 16)], w4_buf.at[c, pl.ds(r0, 16)],
                                          w4_sem.at[c]).start(priority=k)

            _loop(lo, hi, two_pieces)

        x_copy = pltpu.make_async_copy(x_hbm, x_buf, x_sem)
        x_copy.start()
        _loop(0, QD, lambda g: start_all(wq_copies(g)))
        x_copy.wait()
        x = x_buf[...].astype(jnp.float32)
        xn = jnp.broadcast_to(_layernorm(x).astype(jnp.bfloat16), (MR, D))

        def wq_step(g):
            wait_all(wq_copies(g))
            start_all(wq_copies(g + QD))

        def wq_wo_step(g):
            wait_all(wq_copies(g))
            start_all(wo_copies(g - (NQ - QD)))

        _loop(0, NQ - QD, wq_step)
        _loop(NQ - QD, NQ, wq_wo_step)
        _loop(QD, OD, lambda g: start_all(wo_copies(g)))

        row = lax.broadcasted_iota(jnp.int32, (MR, 128), 0)
        col = lax.broadcasted_iota(jnp.int32, (MR, 128), 1)

        def q_panel(c):
            q = _dot(xn, wq_buf[:, pl.ds(m128(c * PAN), PAN)])
            for k in range(PAN // 128):
                t = (PAN // 128) * c + k
                cc = col + 128 * (t % (PW // 128))
                keep = (cc >= row * DH) & (cc < (row + 1) * DH)
                q_buf[t] = jnp.where(keep, q[:, 128 * k:128 * (k + 1)], 0.0).astype(jnp.bfloat16)

        def wo_step(g):
            wait_all(wo_copies(g))

            @pl.when(g + OD < NO)
            def _():
                start_all(wo_copies(g + OD))

            u = g - (NO - 2 * KD + 1)

            @pl.when((u >= 0) & (u % 2 == 0))
            def _():
                kv_start(False, 0, u // 4, u // 2 % 2)

            @pl.when((g % _Q_EVERY == 0) & (g < QPAN * _Q_EVERY))
            def _():
                q_panel(g // _Q_EVERY)

        _loop(0, NO, wo_step)

        prow = lax.broadcasted_iota(jnp.int32, (MR, PW), 0)
        pcol = lax.broadcasted_iota(jnp.int32, (MR, PW), 1)
        own_head = (pcol >= prow * DH) & (pcol < (prow + 1) * DH)
        scale = DH ** -0.5

        def pair_step(j, acc):
            def k_step(p):
                for h in range(2):
                    kv_wait(False, p, h)

                    @pl.when(p < 2)
                    def _():
                        kv_start(False, j, p + 2, h)

                    @pl.when(p >= 2)
                    def _():
                        kv_start(True, j, p - 2, h)

                q = jnp.concatenate([q_buf[(PW // 128) * j + i] for i in range(PW // 128)], axis=1)
                s_buf[p] = _dot(q, k_buf[p].reshape(PW, PAN)) * scale

            _loop(0, NPAN, k_step)

            s = [s_buf[p] for p in range(NPAN)]
            m = jnp.max(jnp.maximum(jnp.maximum(s[0], s[1]), jnp.maximum(s[2], s[3])),
                        axis=-1, keepdims=True)
            e = [jnp.exp(sp - m) for sp in s]
            l = jnp.sum((e[0] + e[1]) + (e[2] + e[3]), axis=-1, keepdims=True)
            for p in range(NPAN):
                p_buf[p] = e[p].astype(jnp.bfloat16)

            def v_step(p, o):
                for h in range(2):
                    kv_wait(True, p, h)

                    @pl.when(p < 2)
                    def _():
                        kv_start(True, j, p + 2, h)

                    @pl.when((p >= 2) & (j + 1 < NP))
                    def _():
                        kv_start(False, j + 1, p - 2, h)

                    @pl.when((p >= 2) & (j + 1 == NP))
                    def _():
                        slot = (p - 2) * 2 + h
                        lo = (N3 + N4) * slot // KD
                        hi = (N3 + N4) * (slot + 1) // KD
                        w3_start(jnp.minimum(lo, N3), jnp.minimum(hi, N3))
                        w4_start(jnp.maximum(lo - N3, 0), jnp.maximum(hi - N3, 0))

                return o + lax.dot_general(
                    p_buf[p], v_buf[p].reshape(PW, PAN), (((1,), (1,)), ((), ())),
                    preferred_element_type=jnp.float32)

            o = lax.fori_loop(0, NPAN, v_step, jnp.zeros((MR, PW), jnp.float32))
            o = jnp.where(own_head, o / l, 0.0).astype(jnp.bfloat16)
            return acc + _dot(o, wo_buf[pl.ds(pl.multiple_of(j * PW, 16), PW), :])

        acc = lax.fori_loop(0, NP, pair_step, jnp.zeros((MR, D), jnp.float32))
        h = x + jnp.sum(acc, axis=0, keepdims=True)

        xb = _layernorm(h)
        y = jnp.broadcast_to(_layernorm(xb).astype(jnp.bfloat16), (MR, D))
        pltpu.make_async_copy(w3_buf, w3_buf, w3_sem).wait()
        g = jax.nn.gelu(_dot(y, w3_buf[...]), approximate=True).astype(jnp.bfloat16)
        for c in range(_W4_CHUNKS):
            g_buf[c] = g[:, c * R4:(c + 1) * R4]

        def w4_step(c, out):
            pltpu.make_async_copy(w4_buf.at[c], w4_buf.at[c], w4_sem.at[c]).wait()
            return out + _dot(g_buf[c], w4_buf[c])

        out = lax.fori_loop(0, _W4_CHUNKS, w4_step, jnp.broadcast_to(h + xb, (MR, D)))
        o_ref[...] = out[0:1].astype(o_ref.dtype)

    return kernel


@jax.jit
def pallas_sequential_preLN__sliding_block_cached__mixer_s_mlp__decode_kernel(
    A_x: jax.Array,
    A_k_cache: jax.Array,
    A_v_cache: jax.Array,
    A_wq: jax.Array,
    A_wo: jax.Array,
    B_x: jax.Array,
    B_w1: jax.Array,
    B_w2: jax.Array,
    B_w3: jax.Array,
    B_w4: jax.Array,
):
    B, Sq, D = A_x.shape
    _, H, SK, DH = A_k_cache.shape
    F = B_w3.shape[1]
    W = min(4096, max(256, SK // 4))
    assert B == 1 and Sq == 1 and H % 2 == 0
    PW, NPAN, R4 = 2 * DH, W // _PAN, F // _W4_CHUNKS

    k_t = jnp.swapaxes(A_k_cache, 2, 3).reshape(H * DH, SK)
    v_t = jnp.swapaxes(A_v_cache, 2, 3).reshape(H * DH, SK)
    bf, f32 = jnp.bfloat16, jnp.float32
    dma = pltpu.SemaphoreType.DMA
    out = pl.pallas_call(
        _make_kernel(D, H, DH, SK, W, F),
        out_shape=jax.ShapeDtypeStruct((1, D), A_x.dtype),
        in_specs=[pl.BlockSpec(memory_space=pl.ANY)] * 7,
        out_specs=pl.BlockSpec(memory_space=pltpu.VMEM),
        scratch_shapes=[
            pltpu.VMEM((1, D), bf),
            pltpu.VMEM((NPAN, PW // 16, 16, _PAN), bf),
            pltpu.VMEM((NPAN, PW // 16, 16, _PAN), bf),
            pltpu.VMEM((D, H * DH), bf),
            pltpu.VMEM((H * DH, D), bf),
            pltpu.VMEM((D, F), bf),
            pltpu.VMEM((_W4_CHUNKS, R4, D), bf),
            pltpu.VMEM((H * DH // 128, _MR, 128), bf),
            pltpu.VMEM((NPAN, _MR, _PAN), f32),
            pltpu.VMEM((NPAN, _MR, _PAN), bf),
            pltpu.VMEM((_W4_CHUNKS, _MR, R4), bf),
            dma(()),
            dma((_Q_DEPTH + 1,)),
            dma((_O_DEPTH + 1,)),
            dma((2, NPAN, 2)),
            dma(()),
            dma((_W4_CHUNKS,)),
        ],
        compiler_params=pltpu.CompilerParams(
            vmem_limit_bytes=64 * 1024 * 1024,
            disable_bounds_checks=True,
            disable_semaphore_checks=True,
        ),
    )(A_x.reshape(1, D), k_t, v_t, A_wq, A_wo, B_w3, B_w4.reshape(_W4_CHUNKS, R4, D))
    return out.reshape(1, 1, D)
```
